```python
import os as _os
_os.environ.setdefault("JAX_PLATFORMS", "cpu")
import jax
import jax.numpy as jnp

def _softmax(x, axis=-1):
    return jax.nn.softmax(x, axis=axis)
def _gelu(x):
    return jax.nn.gelu(x, approximate=True)
def _silu(x):
    return jax.nn.silu(x)
def _sigmoid(x):
    return jax.nn.sigmoid(x)
def _layernorm(x, axis=-1, eps=1e-5):
    m = jnp.mean(x, axis=axis, keepdims=True)
    v = jnp.var(x, axis=axis, keepdims=True)
    return (x - m) / jnp.sqrt(v + eps)
def _scatter_add(tgt, idx, src, axis=0):
    return tgt.at[idx].add(src)
def _segment_sum(src, seg, n):
    return jax.ops.segment_sum(src, seg, n)
class _Rng:
    def __init__(self, key):
        self._k = key
    def _next(self):
        self._k, sub = jax.random.split(self._k)
        return sub
    def normal(self, shape):
        return jax.random.normal(self._next(), shape, dtype=jnp.bfloat16)
    def randint(self, lo, hi, shape):
        return jax.random.randint(self._next(), shape, lo, hi, dtype=jnp.int32)
    def uniform(self, shape, lo=0.0, hi=1.0):
        return jax.random.uniform(self._next(), shape, jnp.bfloat16, lo, hi)
    def permutation(self, n):
        return jax.random.permutation(self._next(), n)


kernel_name = 'concat_heads__gqa_block_cached__mha_block_cached__near_ridge'

def setup_inputs():
    _rng = _Rng(jax.random.key(int.from_bytes(__import__("os").urandom(4), "little")))
    _w = (lambda a: (lambda t: t.astype(jnp.bfloat16) if jnp.issubdtype(t.dtype, jnp.floating) else t)(jnp.asarray(a)))
    def _A_setup():
        B, Sq, D = 16, 32, 1024
        Hq, Hkv, Sk, Dh = 32, 4, 32, 128
        assert Hq % Hkv == 0, (Hq, Hkv)
        return {
            "x": _w((lambda *s: _rng.normal(s) * 0.8)(B, Sq, D)),
            "k_cache": _w((lambda *s: _rng.normal(s) * 0.8)(B, Hkv, Sk, Dh)),
            "v_cache": _w((lambda *s: _rng.normal(s) * 0.05)(B, Hkv, Sk, Dh)),
            "wq": _w((lambda *s: _rng.normal(s) * 0.8)(D, Hq * Dh) * (D ** -0.5)),
            "wo": _w((lambda *s: _rng.normal(s) * 0.05)(Hq * Dh, D) * ((Hq * Dh) ** -0.5)),
        }
    _A_in = _A_setup()

    def _B_setup():
        B, Sq, D = 16, 32, 1024
        H, Sk, Dh = 32, 32, 128
        return {
            "x": _w((lambda *s: _rng.normal(s) * 0.8)(B, Sq, D)),
            "k_cache": _w((lambda *s: _rng.normal(s) * 0.8)(B, H, Sk, Dh)),
            "v_cache": _w((lambda *s: _rng.normal(s) * 0.05)(B, H, Sk, Dh)),
            "wq": _w((lambda *s: _rng.normal(s) * 0.8)(D, H * Dh) * (D ** -0.5)),
            "wo": _w((lambda *s: _rng.normal(s) * 0.05)(H * Dh, D) * ((H * Dh) ** -0.5)),
        }
    _B_in = _B_setup()

    return {
        "A_x": _A_in["x"],
        "A_k_cache": _A_in["k_cache"],
        "A_v_cache": _A_in["v_cache"],
        "A_wq": _A_in["wq"],
        "A_wo": _A_in["wo"],
        "B_x": _B_in["x"],
        "B_k_cache": _B_in["k_cache"],
        "B_v_cache": _B_in["v_cache"],
        "B_wq": _B_in["wq"],
        "B_wo": _B_in["wo"],
    }

def reference(A_x, A_k_cache, A_v_cache, A_wq, A_wo, B_x, B_k_cache, B_v_cache, B_wq, B_wo):
    def _A_ref(x, k_cache, v_cache, wq, wo):
        B, Sq, D = x.shape
        Hq, Dh = 32, 128
        Hkv = k_cache.shape[1]
        rep = Hq // Hkv
        q = (lambda x, *d: x.transpose(*d))((x @ wq).reshape(B, Sq, Hq, Dh), 0, 2, 1, 3)
        k = jnp.repeat(k_cache, rep, axis=1)
        v = jnp.repeat(v_cache, rep, axis=1)
        scores = jnp.einsum("bhqd,bhkd->bhqk", q, k) * (Dh ** -0.5)
        p = _softmax(scores, axis=-1)
        o = jnp.einsum("bhqk,bhkd->bhqd", p, v)
        return (lambda x, *d: x.transpose(*d))(o, 0, 2, 1, 3).reshape(B, Sq, Hq * Dh) @ wo

    def _B_ref(x, k_cache, v_cache, wq, wo):
        B, Sq, D = x.shape
        H, Dh = 32, 128
        q = (lambda x, *d: x.transpose(*d))((x @ wq).reshape(B, Sq, H, Dh), 0, 2, 1, 3)
        scores = jnp.einsum("bhqd,bhkd->bhqk", q, k_cache) * (Dh ** -0.5)
        p = _softmax(scores, axis=-1)
        o = jnp.einsum("bhqk,bhkd->bhqd", p, v_cache)
        return (lambda x, *d: x.transpose(*d))(o, 0, 2, 1, 3).reshape(B, Sq, H * Dh) @ wo

    a = _A_ref(A_x, A_k_cache, A_v_cache, A_wq, A_wo)
    b = _B_ref(B_x, B_k_cache, B_v_cache, B_wq, B_wo)
    return jnp.concatenate([a, b], axis=-1)
```

```python
import jax
import jax.numpy as jnp
from jax import lax
import jax.experimental.pallas as pl
import jax.experimental.pallas.tpu as pltpu

B, SQ, D = 16, 32, 1024
H, SK, DH = 32, 32, 128
HKV_A = 4
M = B * SQ
HI = 8
NI = H // HI
CW = HI * DH
HW = CW // 2
SCALE = DH ** -0.5
BF16 = jnp.bfloat16
F32 = jnp.float32
NT = (((1,), (1,)), ((), ()))

S_X0, S_X1, S_XB = 0, 1, 2
S_P = 3
S_WQ = 7
S_WO = 15
S_K = 23
S_V = 31
S_OUTA = 39
S_OUTB = 40
NSEM = 48


def _recip(l):
    r = pl.reciprocal(l, approx=True)
    return r * (2.0 - l * r)


def kernel(xa_hbm, ka_hbm, va_hbm, wqa_hbm, woa_hbm, xb_hbm, kb_hbm, vb_hbm, wqb_hbm, wob_hbm,
           out_hbm,
           x_buf, wq_buf, wo_buf, ka_buf, va_buf, kb_buf, vb_buf, acc_ref, out_buf, sem):
    wq_hbm = (wqa_hbm, wqb_hbm)
    wo_hbm = (woa_hbm, wob_hbm)

    def cp(src, dst, s):
        return pltpu.make_async_copy(src, dst, sem.at[s])

    def cp_xa(half):
        sl = pl.ds(half * HW, HW)
        return cp(xa_hbm.at[:, sl], x_buf.at[0, :, sl], S_X0 + half)

    def cp_wq0(r0, nr, c0, nc, s):
        return cp(wqa_hbm.at[pl.ds(r0, nr), pl.ds(c0, nc)], wq_buf.at[0, pl.ds(r0, nr), pl.ds(c0, nc)], s)

    p_wq_a = lambda: cp_wq0(0, HW, 0, HW, S_P)
    p_wq_b = lambda: cp_wq0(HW, HW, 0, HW, S_P + 1)
    p_wq_c = lambda: cp_wq0(0, D, HW, 3 * DH, S_P + 2)
    p_wq_d = lambda: cp_wq0(0, D, HW + 3 * DH, DH, S_P + 3)
    p_wo_a = lambda: cp(woa_hbm.at[pl.ds(0, HW), :], wo_buf.at[0, pl.ds(0, HW), :], S_WQ)
    p_wo_b = lambda: cp(woa_hbm.at[pl.ds(HW, HW), :], wo_buf.at[0, pl.ds(HW, HW), :], S_WO)

    def cp_wq(br, j):
        return cp(wq_hbm[br].at[:, pl.ds(j * CW, CW)], wq_buf.at[br * NI + j], S_WQ + br * NI + j)

    def cp_wo(br, j):
        return cp(wo_hbm[br].at[pl.ds(j * CW, CW), :], wo_buf.at[br * NI + j], S_WO + br * NI + j)

    def cp_k(br, j):
        if br == 0:
            return cp(ka_hbm.at[:, pl.ds(j, 1)], ka_buf.at[j], S_K + j)
        return cp(kb_hbm.at[:, pl.ds(j * HI, HI)], kb_buf.at[j], S_K + NI + j)

    def cp_v(br, j):
        if br == 0:
            return cp(va_hbm.at[:, pl.ds(j, 1)], va_buf.at[j], S_V + j)
        return cp(vb_hbm.at[:, pl.ds(j * HI, HI)], vb_buf.at[j], S_V + NI + j)

    cp_xb = lambda: cp(xb_hbm, x_buf.at[1], S_XB)
    cp_outa = lambda: cp(out_buf.at[0], out_hbm.at[:, pl.ds(0, D)], S_OUTA)

    def cp_outb(n):
        return cp(out_buf.at[1, :, pl.ds(n * DH, DH)], out_hbm.at[:, pl.ds(D + n * DH, DH)], S_OUTB + n)

    cp_xa(0).start(); p_wq_a().start()
    cp_xa(1).start(); p_wq_b().start()
    cp_k(0, 0).start(); cp_v(0, 0).start(); p_wq_c().start()
    p_wq_d().start(); p_wo_a().start()
    p_wo_b().start()
    for br in range(2):
        if br == 1:
            cp_xb().start()
        for j in range(1 - br, NI):
            cp_wq(br, j).start(); cp_k(br, j).start(); cp_v(br, j).start(); cp_wo(br, j).start()

    acc_ref[1] = jnp.zeros((M, D), F32)

    def chunk(br, j, first=False):
        c = br * NI + j
        q, p, o, ob = {}, {}, {}, {}

        def Qh(h, half, stage=False):
            part = jnp.dot(x_buf[br, :, half * HW:(half + 1) * HW],
                           wq_buf[c, half * HW:(half + 1) * HW, h * DH:(h + 1) * DH],
                           preferred_element_type=F32)
            if stage:
                if half == 0:
                    acc_ref[br, :, h * DH:(h + 1) * DH] = part
                else:
                    q[h] = (acc_ref[br, :, h * DH:(h + 1) * DH] + part).astype(BF16)
            else:
                q[h] = part if half == 0 else (q[h] + part).astype(BF16)

        def Qp(h):
            Qh(h, 0); Qh(h, 1)

        def Op(sg, n0, n1):
            sl = slice(n0 * DH, n1 * DH)
            ao = jnp.concatenate([o[h] for h in range(4 * sg, 4 * sg + 4)], axis=1)
            r = jnp.dot(ao, wo_buf[c, sg * HW:(sg + 1) * HW, sl], preferred_element_type=F32)
            if not (first and sg == 0):
                r = acc_ref[br, :, sl] + r
            acc_ref[br, :, sl] = r
            if sg == 1 and not first:
                out_buf[br, :, sl] = r.astype(BF16)

        if br == 1:
            rr = lax.broadcasted_iota(jnp.int32, (128, 128), 0) // SQ
            cc = lax.broadcasted_iota(jnp.int32, (128, 128), 1) // SK
            mask = rr == cc

            def kv(ref, h, t):
                return ref[j, 4 * t:4 * t + 4, h].reshape(128, DH)

            def QK(h):
                p[h] = []
                for t in range(4):
                    s = lax.dot_general(q[h][128 * t:128 * (t + 1)], kv(kb_buf, h, t), NT,
                                        preferred_element_type=F32)
                    s = jnp.where(mask, s, -jnp.inf)
                    m = jnp.max(s, axis=-1, keepdims=True)
                    e = jnp.exp((s - m) * SCALE)
                    l = jnp.sum(e, axis=-1, keepdims=True)
                    p[h].append((e * _recip(l)).astype(BF16))

            def PV(h):
                o[h] = jnp.concatenate(
                    [jnp.dot(p[h][t], kv(vb_buf, h, t), preferred_element_type=F32).astype(BF16)
                     for t in range(4)], axis=0)

            Qp(0); Qp(1); QK(0)
            for h in range(2, 8):
                Qp(h); PV(h - 2); QK(h - 1)
            Op(0, 0, 2); PV(6); QK(7)
            Op(0, 2, 4); PV(7)
            Op(0, 4, 8)
            for n in range(8):
                Op(1, n, n + 1)

                @pl.when(j == NI - 1)
                def _():
                    cp_outb(n).start()
        else:
            def QK(sg, t):
                for b in range(4 * t, 4 * t + 4):
                    qs = jnp.concatenate([q[h][SQ * b:SQ * (b + 1)] for h in range(4 * sg, 4 * sg + 4)], axis=0)
                    st = lax.dot_general(ka_buf[j, b, 0], qs, NT, preferred_element_type=F32)
                    m = jnp.max(st, axis=0, keepdims=True)
                    e = jnp.exp((st - m) * SCALE)
                    l = jnp.sum(e, axis=0, keepdims=True)
                    p[sg, b] = (e * _recip(l)).T.astype(BF16)

            def PV(sg, t):
                for b in range(4 * t, 4 * t + 4):
                    ob[sg, b] = jnp.dot(p[sg, b], va_buf[j, b, 0], preferred_element_type=F32).astype(BF16)
                if t == 3:
                    for hh in range(4):
                        o[4 * sg + hh] = jnp.concatenate(
                            [ob[sg, b][SQ * hh:SQ * (hh + 1)] for b in range(B)], axis=0)

            if first:
                cp_xa(0).wait(); p_wq_a().wait()
                for h in range(4):
                    Qh(h, 0, stage=True)
                cp_xa(1).wait(); p_wq_b().wait()
                for h in range(4):
                    Qh(h, 1, stage=True)
                cp_k(0, 0).wait(); cp_v(0, 0).wait(); p_wq_c().wait()
            else:
                Qp(0); Qp(1); Qp(2); Qp(3)
            Qh(4, 0); QK(0, 0); Qh(4, 1); QK(0, 1); Qh(5, 0); QK(0, 2); PV(0, 0); Qh(5, 1); QK(0, 3); PV(0, 1)
            Qh(6, 0); PV(0, 2); Qh(6, 1)
            if first:
                p_wq_d().wait(); p_wo_a().wait()
            PV(0, 3); Qh(7, 0); Qh(7, 1)
            Op(0, 0, 1); QK(1, 0); Op(0, 1, 2); QK(1, 1); Op(0, 2, 3); QK(1, 2); PV(1, 0)
            Op(0, 3, 4); QK(1, 3); PV(1, 1)
            Op(0, 4, 5); PV(1, 2); Op(0, 5, 6); PV(1, 3); Op(0, 6, 8)
            if first:
                p_wo_b().wait()
            Op(1, 0, 8)

    chunk(0, 0, first=True)

    def body(br):
        def f(j, carry):
            cp_wq(br, j).wait(); cp_k(br, j).wait(); cp_v(br, j).wait(); cp_wo(br, j).wait()
            chunk(br, j)
            return carry
        return f

    lax.fori_loop(1, NI, body(0), 0)
    cp_outa().start()
    cp_xb().wait()
    lax.fori_loop(0, NI, body(1), 0)
    cp_outa().wait()
    for n in range(8):
        cp_outb(n).wait()


@jax.jit
def pallas_concat_heads__gqa_block_cached__mha_block_cached__near_ridge_kernel(
    A_x, A_k_cache, A_v_cache, A_wq, A_wo, B_x, B_k_cache, B_v_cache, B_wq, B_wo,
):
    xa = A_x.reshape(M, D)
    xb = B_x.reshape(M, D)
    any_spec = pl.BlockSpec(memory_space=pl.ANY)
    out = pl.pallas_call(
        kernel,
        in_specs=[any_spec] * 10,
        out_specs=any_spec,
        out_shape=jax.ShapeDtypeStruct((M, 2 * D), BF16),
        scratch_shapes=[
            pltpu.VMEM((2, M, D), BF16),
            pltpu.VMEM((2 * NI, D, CW), BF16),
            pltpu.VMEM((2 * NI, CW, D), BF16),
            pltpu.VMEM((NI, B, 1, SK, DH), BF16),
            pltpu.VMEM((NI, B, 1, SK, DH), BF16),
            pltpu.VMEM((NI, B, HI, SK, DH), BF16),
            pltpu.VMEM((NI, B, HI, SK, DH), BF16),
            pltpu.VMEM((2, M, D), F32),
            pltpu.VMEM((2, M, D), BF16),
            pltpu.SemaphoreType.DMA((NSEM,)),
        ],
        compiler_params=pltpu.CompilerParams(
            vmem_limit_bytes=100 * 1024 * 1024,
        ),
    )(xa, A_k_cache, A_v_cache, A_wq, A_wo, xb, B_k_cache, B_v_cache, B_wq, B_wo)
    return out.reshape(B, SQ, 2 * D)
```

```python
import jax
import jax.numpy as jnp
from jax import lax
import jax.experimental.pallas as pl
import jax.experimental.pallas.tpu as pltpu

B, SQ, D = 16, 32, 1024
H, SK, DH = 32, 32, 128
M = B * SQ
HI = 8
NI = H // HI
CW = HI * DH
HW = CW // 2
PAD = 128
SCALE = DH ** -0.5
BF16 = jnp.bfloat16
F32 = jnp.float32
NT = (((1,), (1,)), ((), ()))

KSPLIT = (128, 128, 256)
LASTQ = 4
NST = 7
S_XO = 7
NSEM = 8


def _recip(l):
    r = pl.reciprocal(l, approx=True)
    return r * (2.0 - l * r)


def _kernel(xa_hbm, ka_hbm, va_hbm, wqa_hbm, woa_hbm, xb_hbm, kb_hbm, vb_hbm, wqb_hbm, wob_hbm,
            out_hbm,
            x_buf, wq_buf, wo_buf, ka_buf, va_buf, kb_buf, vb_buf, acc_ref, out_buf, sem):
    wq_hbm = (wqa_hbm, wqb_hbm)
    wo_hbm = (woa_hbm, wob_hbm)

    def cp(src, dst, s):
        return pltpu.make_async_copy(src, dst, sem.at[s])

    def cp_xa(k0, nk, s):
        return cp(xa_hbm.at[:, pl.ds(k0, nk)], x_buf.at[0, :, pl.ds(k0, nk)], s)

    def cp_wq0(r0, nr, c0, nc, s):
        return cp(wqa_hbm.at[pl.ds(r0, nr), pl.ds(c0, nc)], wq_buf.at[0, pl.ds(r0, nr), pl.ds(c0, nc)], s)

    def cp_wo0(r0, s):
        return cp(woa_hbm.at[pl.ds(r0, HW), :], wo_buf.at[0, pl.ds(r0, HW), pl.ds(0, D)], s)

    def cp_kv(br, j, s):
        if br == 0:
            return [cp(ka_hbm.at[:, pl.ds(j, 1)], ka_buf.at[j], s),
                    cp(va_hbm.at[:, pl.ds(j, 1)], va_buf.at[j], s)]
        return [cp(kb_hbm.at[:, pl.ds(j * HI, HI)], kb_buf.at[j], s),
                cp(vb_hbm.at[:, pl.ds(j * HI, HI)], vb_buf.at[j], s)]

    def stage(i):
        if i < 3:
            k0, nk = sum(KSPLIT[:i]), KSPLIT[i]
            return [cp_xa(k0, nk, i), cp_wq0(k0, nk, 0, CW, i)]
        if i == 3:
            return [cp_xa(HW, HW, i), cp_wq0(HW, HW, 0, HW, i)]
        if i == 4:
            return cp_kv(0, 0, i) + [cp_wq0(HW, HW, HW, HW, i)]
        return [cp_wo0((i - 5) * HW, i)]

    def chunk_copies(br, j):
        c = br * NI + j
        return ([cp(wq_hbm[br].at[:, pl.ds(j * CW, CW)], wq_buf.at[c, :, pl.ds(0, CW)], c - 1)]
                + cp_kv(br, j, c - 1)
                + [cp(wo_hbm[br].at[pl.ds(j * CW, CW), :], wo_buf.at[c, :, pl.ds(0, D)], c - 1)])

    def start(cs):
        for c in cs:
            c.start()

    def wait(cs):
        for c in cs:
            c.wait()

    def cp_xb():
        return cp(xb_hbm, x_buf.at[1], S_XO)

    def cp_outa():
        return cp(out_buf.at[0], out_hbm.at[:, pl.ds(0, D)], S_XO)

    def cp_outb(n, r0, nr):
        return cp(out_buf.at[1, pl.ds(r0, nr), pl.ds(n * DH, DH)],
                  out_hbm.at[pl.ds(r0, nr), pl.ds(D + n * DH, DH)], S_XO)

    def chunk(br, j, first=False, emit=True):
        c = br * NI + j
        q, p, o, ob = {}, {}, {}, {}

        def Qp(h):
            cols = slice(h * DH, (h + 1) * DH)
            if first:
                part = jnp.dot(x_buf[br, :, HW:], wq_buf[c, HW:, cols], preferred_element_type=F32)
                q[h] = (acc_ref[br, :, cols] + part).astype(BF16)
            else:
                q[h] = jnp.dot(x_buf[br], wq_buf[c, :, cols], preferred_element_type=F32).astype(BF16)

        def Qr(h, half):
            part = jnp.dot(x_buf[br, half * (M // 2):(half + 1) * (M // 2), :],
                           wq_buf[c, :, h * DH:(h + 1) * DH], preferred_element_type=F32).astype(BF16)
            q[h] = part if half == 0 else jnp.concatenate([q[h], part], axis=0)

        def Op(sg, n0, n1):
            cols = slice(n0 * DH, n1 * DH)
            ao = jnp.concatenate([o[h] for h in range(4 * sg, 4 * sg + 4)], axis=1)
            r = jnp.dot(ao, wo_buf[c, sg * HW:(sg + 1) * HW, cols], preferred_element_type=F32)
            if not (first and sg == 0):
                r = acc_ref[br, :, cols] + r
            acc_ref[br, :, cols] = r
            return r

        if br == 1:
            rr = lax.broadcasted_iota(jnp.int32, (128, 128), 0) // SQ
            cc = lax.broadcasted_iota(jnp.int32, (128, 128), 1) // SK
            mask = rr == cc

            def kv(ref, h, t):
                return ref[j, 4 * t:4 * t + 4, h].reshape(4 * SK, DH)

            def QK(h):
                p[h] = []
                for t in range(4):
                    s = lax.dot_general(q[h][128 * t:128 * (t + 1)], kv(kb_buf, h, t), NT,
                                        preferred_element_type=F32)
                    s = jnp.where(mask, s, -jnp.inf)
                    m = jnp.max(s, axis=-1, keepdims=True)
                    e = jnp.exp((s - m) * SCALE)
                    l = jnp.sum(e, axis=-1, keepdims=True)
                    p[h].append((e * _recip(l)).astype(BF16))

            def PV(h):
                o[h] = jnp.concatenate(
                    [jnp.dot(p[h][t], kv(vb_buf, h, t), preferred_element_type=F32).astype(BF16)
                     for t in range(4)], axis=0)

            Qp(0); Qp(1); QK(0)
            for h in range(2, HI):
                Qp(h); PV(h - 2); QK(h - 1)
            Op(0, 0, 2); PV(6); QK(7)
            Op(0, 2, 4); PV(7)
            Op(0, 4, 8)
            if not emit:
                Op(1, 0, 8)
                return
            for n in range(8):
                r = Op(1, n, n + 1).astype(BF16)
                nq = LASTQ if n == 7 else 1
                for i in range(nq):
                    r0, nr = i * (M // nq), M // nq
                    out_buf[1, r0:r0 + nr, n * DH:(n + 1) * DH] = r[r0:r0 + nr]

                    @pl.when(j == NI - 1)
                    def _():
                        cp_outb(n, r0, nr).start()
            return

        def QK(sg, t):
            for b in range(4 * t, 4 * t + 4):
                qs = jnp.concatenate([q[h][SQ * b:SQ * (b + 1)] for h in range(4 * sg, 4 * sg + 4)], axis=0)
                st = lax.dot_general(ka_buf[j, b, 0], qs, NT, preferred_element_type=F32)
                m = jnp.max(st, axis=0, keepdims=True)
                e = jnp.exp((st - m) * SCALE)
                l = jnp.sum(e, axis=0, keepdims=True)
                p[sg, b] = (e * _recip(l)).T.astype(BF16)

        def PV(sg, t):
            for b in range(4 * t, 4 * t + 4):
                ob[sg, b] = jnp.dot(p[sg, b], va_buf[j, b, 0], preferred_element_type=F32).astype(BF16)
            if t == 3:
                for hh in range(4):
                    o[4 * sg + hh] = jnp.concatenate(
                        [ob[sg, b][SQ * hh:SQ * (hh + 1)] for b in range(B)], axis=0)

        if first:
            for i, nk in enumerate(KSPLIT):
                k0 = sum(KSPLIT[:i])
                wait(stage(i))
                r = jnp.dot(x_buf[0, :, k0:k0 + nk], wq_buf[0, k0:k0 + nk, 0:CW], preferred_element_type=F32)
                acc_ref[0] = r if i == 0 else acc_ref[0] + r
            for jj in range(1, NI):
                start(chunk_copies(0, jj))
            cp_xb().start()
            wait(stage(3))
            Qp(0); Qp(1); Qp(2); Qp(3)
            wait(stage(4))
            Qp(4); QK(0, 0); QK(0, 1); Qp(5); QK(0, 2); PV(0, 0); QK(0, 3); PV(0, 1)
            Qp(6); PV(0, 2); PV(0, 3); Qp(7)
            wait(stage(5))
        else:
            Qp(0); Qp(1); Qp(2); Qp(3)
            Qr(4, 0); QK(0, 0); Qr(4, 1); QK(0, 1); Qr(5, 0); QK(0, 2); PV(0, 0); Qr(5, 1); QK(0, 3); PV(0, 1)
            Qp(6); PV(0, 2); PV(0, 3); Qp(7)
        Op(0, 0, 1); QK(1, 0); Op(0, 1, 2); QK(1, 1); Op(0, 2, 3); QK(1, 2); PV(1, 0)
        Op(0, 3, 4); QK(1, 3); PV(1, 1); Op(0, 4, 5); PV(1, 2); Op(0, 5, 6); PV(1, 3); Op(0, 6, 8)
        if first:
            wait(stage(6))
            Op(1, 0, 8)
            for jj in range(NI):
                start(chunk_copies(1, jj))
        else:
            out_buf[0] = Op(1, 0, 8).astype(BF16)

    for i in range(NST):
        start(stage(i))
    acc_ref[1] = jnp.zeros((M, D), F32)

    def body_a(j, carry):
        wait(chunk_copies(0, j))
        chunk(0, j)
        return carry

    def body_b(i, carry):
        wait(chunk_copies(1, 2 * i) + chunk_copies(1, 2 * i + 1))
        chunk(1, 2 * i, emit=False)
        chunk(1, 2 * i + 1)
        return carry

    def branch(br, carry):
        @pl.when(br == 0)
        def _():
            chunk(0, 0, first=True)
            lax.fori_loop(1, NI, body_a, 0)

        @pl.when(br == 1)
        def _():
            cp_xb().wait()
            cp_outa().start()
            lax.fori_loop(0, NI // 2, body_b, 0)
        return carry

    lax.fori_loop(0, 2, branch, 0)
    cp(out_hbm, out_hbm, S_XO).wait()


@jax.jit
def pallas_concat_heads__gqa_block_cached__mha_block_cached__near_ridge_kernel(
    A_x: jax.Array,
    A_k_cache: jax.Array,
    A_v_cache: jax.Array,
    A_wq: jax.Array,
    A_wo: jax.Array,
    B_x: jax.Array,
    B_k_cache: jax.Array,
    B_v_cache: jax.Array,
    B_wq: jax.Array,
    B_wo: jax.Array,
):
    any_spec = pl.BlockSpec(memory_space=pl.ANY)
    out = pl.pallas_call(
        _kernel,
        in_specs=[any_spec] * 10,
        out_specs=any_spec,
        out_shape=jax.ShapeDtypeStruct((M, 2 * D), BF16),
        scratch_shapes=[
            pltpu.VMEM((2, M, D), BF16),
            pltpu.VMEM((2 * NI, D, CW + PAD), BF16),
            pltpu.VMEM((2 * NI, CW, D + PAD), BF16),
            pltpu.VMEM((NI, B, 1, SK, DH), BF16),
            pltpu.VMEM((NI, B, 1, SK, DH), BF16),
            pltpu.VMEM((NI, B, HI, SK, DH), BF16),
            pltpu.VMEM((NI, B, HI, SK, DH), BF16),
            pltpu.VMEM((2, M, D), F32),
            pltpu.VMEM((2, M, D), BF16),
            pltpu.SemaphoreType.DMA((NSEM,)),
        ],
        compiler_params=pltpu.CompilerParams(
            vmem_limit_bytes=100 * 1024 * 1024,
        ),
    )(A_x.reshape(M, D), A_k_cache, A_v_cache, A_wq, A_wo,
      B_x.reshape(M, D), B_k_cache, B_v_cache, B_wq, B_wo)
    return out.reshape(B, SQ, 2 * D)
```
